```python
import os as _os
_os.environ.setdefault("JAX_PLATFORMS", "cpu")
import jax
import jax.numpy as jnp

def _softmax(x, axis=-1):
    return jax.nn.softmax(x, axis=axis)
def _gelu(x):
    return jax.nn.gelu(x, approximate=True)
def _silu(x):
    return jax.nn.silu(x)
def _sigmoid(x):
    return jax.nn.sigmoid(x)
def _layernorm(x, axis=-1, eps=1e-5):
    m = jnp.mean(x, axis=axis, keepdims=True)
    v = jnp.var(x, axis=axis, keepdims=True)
    return (x - m) / jnp.sqrt(v + eps)
def _scatter_add(tgt, idx, src, axis=0):
    return tgt.at[idx].add(src)
def _segment_sum(src, seg, n):
    return jax.ops.segment_sum(src, seg, n)
class _Rng:
    def __init__(self, key):
        self._k = key
    def _next(self):
        self._k, sub = jax.random.split(self._k)
        return sub
    def normal(self, shape):
        return jax.random.normal(self._next(), shape, dtype=jnp.bfloat16)
    def randint(self, lo, hi, shape):
        return jax.random.randint(self._next(), shape, lo, hi, dtype=jnp.int32)
    def uniform(self, shape, lo=0.0, hi=1.0):
        return jax.random.uniform(self._next(), shape, jnp.bfloat16, lo, hi)
    def permutation(self, n):
        return jax.random.permutation(self._next(), n)


kernel_name = 'concat_heads__spectral_gfnet__mha_block__prompt'

def setup_inputs():
    _rng = _Rng(jax.random.key(int.from_bytes(__import__("os").urandom(4), "little")))
    _w = (lambda a: (lambda t: t.astype(jnp.bfloat16) if jnp.issubdtype(t.dtype, jnp.floating) else t)(jnp.asarray(a)))
    def _A_setup():
        B, S, D = 1, 2048, 576
        Df = D // 2 + 1
        return {
            "x": _w((lambda *s: _rng.normal(s) * 0.05)(B, S, D)),
            "w_r": _w((lambda *s: _rng.normal(s) * 0.05)(S, Df) * 0.02),
            "w_i": _w((lambda *s: _rng.normal(s) * 0.05)(S, Df) * 0.02),
        }
    _A_in = _A_setup()

    def _B_setup():
        B, S, D, H = 1, 2048, 576, 32
        return {
            "x": _w((lambda *s: _rng.normal(s) * 0.1)(B, S, D)),
            "wqkv": _w((lambda *s: _rng.normal(s) * 0.1)(D, 3 * D)),
            "wo": _w((lambda *s: _rng.normal(s) * 0.05)(D, D)),
        }
    _B_in = _B_setup()

    return {
        "A_x": _A_in["x"],
        "A_w_r": _A_in["w_r"],
        "A_w_i": _A_in["w_i"],
        "B_x": _B_in["x"],
        "B_wqkv": _B_in["wqkv"],
        "B_wo": _B_in["wo"],
    }

def reference(A_x, A_w_r, A_w_i, B_x, B_wqkv, B_wo):
    def _A_ref(x, w_r, w_i):
        B, S, D = x.shape
        X = (lambda x, axes=(-2,-1): jnp.fft.rfft2(x.astype(jnp.float32), axes=axes))(x, axes=(-2, -1))
        W = w_r + 1j * w_i
        X = X * W
        y = (lambda x, s, axes=(-2,-1): jnp.fft.irfft2(x, s=s, axes=axes).astype(jnp.bfloat16))(X, (S, D), axes=(-2, -1))
        return y

    def _B_ref(x, wqkv, wo):
        B, S, D = x.shape
        H = 32
        Dh = D // H
        qkv = (lambda x, *d: x.transpose(*d))((x @ wqkv).reshape(B, S, 3, H, Dh), 2, 0, 3, 1, 4)
        q, k, v = qkv[0], qkv[1], qkv[2]
        scores = jnp.einsum("bhqd,bhkd->bhqk", q, k) * (Dh ** -0.5)
        p = _softmax(scores, axis=-1)
        o = jnp.einsum("bhqk,bhkd->bhqd", p, v)
        return (lambda x, *d: x.transpose(*d))(o, 0, 2, 1, 3).reshape(B, S, D) @ wo

    a = _A_ref(A_x, A_w_r, A_w_i)
    b = _B_ref(B_x, B_wqkv, B_wo)
    return jnp.concatenate([a, b], axis=-1)
```

```python
import math

import numpy as np
import jax
import jax.numpy as jnp
from jax import lax
import jax.experimental.pallas as pl
import jax.experimental.pallas.tpu as pltpu

S = 2048
D = 576
H = 32
DH = D // H
DF = D // 2 + 1
LANE = 128

HOLE = DH + 1
KT = LANE - HOLE
NT = -(-S // KT)
SP = NT * LANE
HPB = LANE // DH
NB = -(-H // HPB)
DP = NB * LANE

RC = 512
NPC = 4
PC = RC // NPC
FENCE0 = 6
FENCED = 4
assert S == 4 * RC

R9 = 9
M = D // R9
NG = 5
FR = 296
FP = 384
F2 = 256
FT = FR - F2
N1 = 16
N2 = S // N1
RB = 512
NBK = S // RB
RO = 256
R5 = 64

BF16 = jnp.bfloat16
F32 = jnp.float32


def _group_bins(r):
    if r == 0:
        return [R9 * g for g in range(D // 2 // R9 + 1)]
    return [r + R9 * g for g in range(32)] + [R9 - r + R9 * g for g in range(32)]


def _fft_constants():
    b = np.arange(M, dtype=np.float64)
    scale = 1.0 / (S * D)
    m1 = np.zeros((NG, 2 * M, 2 * M), np.float64)
    m2 = np.zeros((NG, 2 * M, 2 * M), np.float64)
    for r in range(NG):
        bins = _group_bins(r)
        nb = len(bins)
        half = FT if r == 0 else M
        for i, f in enumerate(bins):
            th = 2.0 * np.pi * ((f * b) % D) / D
            c, sn = np.cos(th), np.sin(th)
            sg = 1.0 if (f % R9) == r else -1.0
            m1[r, i, :M] = c
            m1[r, i, M:] = sg * sn
            m1[r, half + i, :M] = -sn
            m1[r, half + i, M:] = sg * c
            cf = (1.0 if f in (0, D // 2) else 2.0) * scale
            swap = r in (2, 4)
            kr = M + i if swap else i
            ki = i if swap else M + i
            if r == 0:
                for k, v in ((kr, cf * c), (ki, -cf * sn)):
                    m2[r, k, :M] = v
                    m2[r, k, M:2 * M] = v
            else:
                for k, vre, vim in ((kr, cf * c, sg * cf * sn), (ki, -cf * sn, sg * cf * c)):
                    m2[r, k, :M] = vre
                    m2[r, k, M:2 * M] = vim
        assert nb <= half

    n2 = np.arange(N2, dtype=np.float64)
    k2 = np.arange(N2, dtype=np.float64)
    g = np.zeros((N1, 2 * N2, 2 * N2), np.float64)
    gi = np.zeros((N1, 2 * N2, 2 * N2), np.float64)
    for k1 in range(N1):
        a = 2.0 * np.pi * ((n2[None, :] * (N1 * k2[:, None] + k1)) % S) / S
        gr_, gi_ = np.cos(a), -np.sin(a)
        g[k1, :N2, :N2] = gr_
        g[k1, :N2, N2:] = -gi_
        g[k1, N2:, :N2] = gi_
        g[k1, N2:, N2:] = gr_
        gi[k1] = g[k1].T
    to = lambda m: jnp.asarray(m.astype(np.float32), dtype=BF16)
    return to(m1), to(m2), to(g), to(gi)


def _cmul_const(a, wr, wi):
    ar, ai = a
    eps = 1e-12
    if abs(wi) < eps:
        return (ar, ai) if wr > 0 else (-ar, -ai)
    if abs(wr) < eps:
        return (-ai, ar) if wi > 0 else (ai, -ar)
    if abs(abs(wr) - abs(wi)) < eps:
        s = abs(wr)
        sr = 1.0 if wr > 0 else -1.0
        si = 1.0 if wi > 0 else -1.0
        if sr * si > 0:
            re, im = (ar - ai), (ar + ai)
            return (re * (s * sr), im * (s * sr))
        re, im = (ar + ai), (ai - ar)
        return (re * (s * sr), im * (s * sr))
    return (ar * wr - ai * wi, ar * wi + ai * wr)


def _fft_small(xs, sign):
    n = len(xs)
    if n == 1:
        return xs
    ev = _fft_small(xs[0::2], sign)
    od = _fft_small(xs[1::2], sign)
    out = [None] * n
    for k in range(n // 2):
        ang = sign * 2.0 * math.pi * k / n
        tr, ti = _cmul_const(od[k], math.cos(ang), math.sin(ang))
        er, ei = ev[k]
        out[k] = (er + tr, ei + ti)
        out[k + n // 2] = (er - tr, ei - ti)
    return out


_NT_DIMS = (((1,), (1,)), ((), ()))


def _kernel(axt_hbm, wrt_hbm, wit_hbm, bxt_hbm, wqkv_hbm, wo_hbm,
            m1_hbm, m2_hbm, g_hbm, gi_hbm,
            out_hbm,
            axt_ref, wrt_ref, wit_ref, bxt_ref, wqkv_ref, wo_ref,
            m1_ref, m2_ref, g_ref, gi_ref, out_ref,
            sem_bx, sem_in, sem_out,
            zt_ref, ar_ref, wtmp_ref, a_ref, t_ref, z_ref, wf_ref,
            x_ref, xp_ref, wq_ref, wv_ref, wkt_ref, wop_ref,
            q_ref, v_ref, w_ref, s_ref, m_ref, mx_ref,
            qc_ref, attn_ref):
    def bx_copy(i):
        cols = pl.ds(pl.multiple_of(i * RB, RB), RB)
        return pltpu.make_async_copy(bxt_hbm.at[:, cols], bxt_ref.at[:, cols], sem_bx.at[i])

    wq_cols = pl.ds(0, DP)
    wkv_cols = pl.ds(DP, 3 * D - DP)
    in_pairs = [(wqkv_hbm.at[:, wq_cols], wqkv_ref.at[:, wq_cols]),
                (wqkv_hbm.at[:, wkv_cols], wqkv_ref.at[:, wkv_cols]),
                (wo_hbm, wo_ref.at[pl.ds(0, D)]),
                (axt_hbm, axt_ref), (wrt_hbm, wrt_ref), (wit_hbm, wit_ref),
                (m1_hbm, m1_ref), (m2_hbm, m2_ref), (g_hbm, g_ref), (gi_hbm, gi_ref)]
    in_copy = [pltpu.make_async_copy(src, dst, sem_in.at[k])
               for k, (src, dst) in enumerate(in_pairs)]
    CP_WQ, CP_WKV, CP_WO = range(3)
    CP_FFT1 = range(3, 7)
    CP_FFT2 = range(7, len(in_pairs))

    in_copy[CP_WQ].start()
    bx_copy(0).start()

    attn_ref[...] = jnp.zeros(attn_ref.shape, BF16)
    wq_ref[:D, :] = jnp.zeros((D, DP), BF16)
    wv_ref[:D, :] = jnp.zeros((D, DP), BF16)
    wop_ref[...] = jnp.zeros(wop_ref.shape, BF16)
    for k1 in range(N1):
        a_ref[k1, FR:F2 + 64, :] = jnp.zeros((F2 + 64 - FR, 2 * N2), F32)
        a_ref[k1, F2 + 64 + FT:, :] = jnp.zeros((FP - F2 - 64 - FT, 2 * N2), F32)

    bx_copy(1).start()
    in_copy[CP_WKV].start()
    for i in range(2, NBK):
        bx_copy(i).start()
    in_copy[CP_WO].start()

    blocks = [(b, b * HPB * DH, min(HPB * DH, D - b * HPB * DH)) for b in range(NB)]
    in_copy[CP_WQ].wait()
    for b, c0, n in blocks:
        wq_ref[:D, b * LANE:b * LANE + n] = wqkv_ref[:, c0:c0 + n]

    qscale = (DH ** -0.5) * math.log2(math.e)

    def b1(i, c):
        bx_copy(i).wait()

        @pl.when(i == NBK - 2)
        def _():
            for k in CP_FFT1:
                in_copy[k].start()
        rows = pl.ds(pl.multiple_of(i * RB, RB), RB)
        x = bxt_ref[:, rows].T
        x_ref[rows, :] = x
        q = jnp.dot(x, wq_ref[:D, :], preferred_element_type=F32) * qscale
        for b in range(NB):
            q_ref[b, rows, :] = q[:, b * LANE:(b + 1) * LANE].astype(BF16)
        return c
    lax.fori_loop(0, NBK, b1, 0)

    in_copy[CP_WKV].wait()
    in_copy[CP_WO].wait()
    for b, c0, n in blocks:
        wv_ref[:D, b * LANE:b * LANE + n] = wqkv_ref[:, 2 * D + c0:2 * D + c0 + n]
        wop_ref[b * LANE:b * LANE + n, DP - D:] = wo_ref[c0:c0 + n, :]
    wkt_ref[:D, :] = wqkv_ref[:, D:2 * D].T

    for j in range(NT):
        xp_ref[j * LANE:j * LANE + HOLE, :] = jnp.zeros((HOLE, D), BF16)
        k0 = j * KT
        n = min(KT, S - k0)
        xp_ref[j * LANE + HOLE:j * LANE + HOLE + n, :] = x_ref[k0:k0 + n, :]
        if n < KT:
            xp_ref[j * LANE + HOLE + n:(j + 1) * LANE, :] = x_ref[0:KT - n, :]

    cs9 = [[math.cos(2.0 * math.pi * r * a / R9) for a in range(R9)] for r in range(NG)]
    sn9 = [[math.sin(2.0 * math.pi * r * a / R9) for a in range(R9)] for r in range(NG)]

    def a1(i):
        lc = slice(i * LANE, (i + 1) * LANE)
        for bb in range(M // 16):
            xs = [axt_ref[a * M + bb * 16:a * M + (bb + 1) * 16, lc].astype(F32)
                  for a in range(R9)]
            ps = [xs[a] + xs[R9 - a] for a in range(1, NG)]
            qs = [xs[a] - xs[R9 - a] for a in range(1, NG)]
            rr = slice(bb * 16, (bb + 1) * 16)
            ri = slice(M + bb * 16, M + (bb + 1) * 16)
            ar_ref[0, rr, :] = (xs[0] + ((ps[0] + ps[1]) + (ps[2] + ps[3]))).astype(BF16)
            for r in range(1, NG):
                re = xs[0]
                im = None
                for a in range(1, NG):
                    re = re + ps[a - 1] * cs9[r][a]
                    t = qs[a - 1] * (-sn9[r][a])
                    im = t if im is None else im + t
                ar_ref[r, rr, :] = re.astype(BF16)
                ar_ref[r, ri, :] = im.astype(BF16)
        for r in range(1, NG):
            zz = jnp.dot(m1_ref[r], ar_ref[r], preferred_element_type=F32)
            zt_ref[(r - 1) * M:r * M, lc] = zz[:M]
            zt_ref[FR + (r - 1) * M:FR + r * M, lc] = zz[M:]
        zz = jnp.dot(m1_ref[0, :2 * FT, :M], ar_ref[0, :M, :], preferred_element_type=F32)
        zt_ref[F2:FR, lc] = zz[:FT]
        zt_ref[FR + F2:, lc] = zz[FT:]
        for part, src in enumerate((wrt_ref, wit_ref)):
            wtmp_ref[part, :DF, :] = src[:, lc].astype(F32)

            def grp(r):
                return [wtmp_ref[part, pl.ds(r, 32, stride=R9), :],
                        wtmp_ref[part, pl.ds(R9 - r, 32, stride=R9), :]]
            g0 = wtmp_ref[part, pl.ds(0, 33, stride=R9), :]
            pad = jnp.zeros((M - 33, LANE), F32)
            tiles = [grp(1) + grp(2), grp(3) + grp(4), [g0, pad, g0, pad]]
            for lt in range(FP // LANE):
                wf_ref[part, lt, lc, :] = jnp.concatenate(tiles[lt], axis=0).T

    def a2_group(r0, dup):
        xs = []
        for n1 in range(N1):
            xs.append((zt_ref[pl.ds(r0, 8), n1 * N2:(n1 + 1) * N2],
                       zt_ref[pl.ds(FR + r0, 8), n1 * N2:(n1 + 1) * N2]))
        ys = _fft_small(xs, -1.0)
        for k1 in range(N1):
            a_ref[k1, pl.ds(r0, 8), :N2] = ys[k1][0]
            a_ref[k1, pl.ds(r0, 8), N2:] = ys[k1][1]
            if dup:
                a_ref[k1, pl.ds(r0 + 64, 8), :N2] = ys[k1][0]
                a_ref[k1, pl.ds(r0 + 64, 8), N2:] = ys[k1][1]

    def a3_one(k1):
        y = lax.dot_general(g_ref[k1], a_ref[k1].astype(BF16), _NT_DIMS,
                            preferred_element_type=F32)
        yr, yi = y[:N2], y[N2:]
        wr = jnp.concatenate([wf_ref[0, lt, pl.ds(k1, N2, stride=N1), :]
                              for lt in range(FP // LANE)], axis=1)
        wi = jnp.concatenate([wf_ref[1, lt, pl.ds(k1, N2, stride=N1), :]
                              for lt in range(FP // LANE)], axis=1)
        p = jnp.concatenate([yr * wr - yi * wi, yr * wi + yi * wr], axis=0).astype(BF16)
        t_ref[k1] = jnp.dot(gi_ref[k1], p, preferred_element_type=F32)

    low8 = lax.broadcasted_iota(jnp.int32, (8, LANE), 1) < M

    def a4(i):
        r0 = pl.multiple_of(i * 8, 8)
        for lt in range(FP // LANE):
            xs = []
            for k1 in range(N1):
                xs.append((t_ref[k1, pl.ds(r0, 8), lt * LANE:(lt + 1) * LANE],
                           t_ref[k1, pl.ds(N2 + r0, 8), lt * LANE:(lt + 1) * LANE]))
            ys = _fft_small(xs, 1.0)
            for n1 in range(N1):
                rr = pl.ds(n1 * N2 + r0, 8)
                ur, ui = ys[n1]
                if lt < 2:
                    uis = pltpu.roll(ui, M, 1)
                    z_ref[rr, 2 * lt * LANE:(2 * lt + 1) * LANE] = jnp.where(low8, ur, uis)
                    z_ref[rr, (2 * lt + 1) * LANE:(2 * lt + 2) * LANE] = jnp.where(low8, uis, ur)
                else:
                    z_ref[rr, 4 * LANE:] = jnp.where(low8, ur, ui)

    low1 = lax.broadcasted_iota(jnp.int32, (1, LANE), 1) < M

    def halves(lo, hi):
        return jnp.where(low1, lo, hi).astype(F32)

    def a5(rows, yb_fn):
        t0 = jnp.dot(z_ref[rows, 4 * LANE:].astype(BF16), m2_ref[0],
                     preferred_element_type=F32)
        ts = [jnp.dot(z_ref[rows, (r - 1) * LANE:r * LANE].astype(BF16), m2_ref[r],
                      preferred_element_type=F32) for r in range(1, NG)]
        tw = [pltpu.roll(t, M, 1) for t in ts]
        for t in range(NB):
            alo, ahi = 2 * t, 2 * t + 1
            has_hi = ahi < R9
            y = t0 if has_hi else t0 * halves(1.0, 0.0)
            for r in range(1, NG):
                al = halves(cs9[r][alo], -sn9[r][ahi] if has_hi else 0.0)
                be = halves(-sn9[r][alo], cs9[r][ahi] if has_hi else 0.0)
                y = y + ts[r - 1] * al + tw[r - 1] * be
            if not has_hi:
                y = y + yb_fn()
            out_ref[rows, t * LANE:(t + 1) * LANE] = y.astype(BF16)

    lane_t = lax.broadcasted_iota(jnp.int32, (LANE, LANE), 1)
    row_t = lax.broadcasted_iota(jnp.int32, (LANE, LANE), 0)
    row24 = lax.broadcasted_iota(jnp.int32, (24, LANE), 0)

    for k in CP_FFT1:
        in_copy[k].wait()
    for k in CP_FFT2:
        in_copy[k].start()

    a2_units = [(r0, r0 >= F2) for r0 in range(0, FR, 8)]
    a2_split = -(-len(a2_units) // (NT - N1))

    def b2(j):
        xt = xp_ref[j * LANE:(j + 1) * LANE, :]
        v = jnp.dot(xt, wv_ref[:D, :], preferred_element_type=F32)
        kt = lax.dot_general(wkt_ref[:D, :], xt, _NT_DIMS, preferred_element_type=F32)
        kt = jnp.concatenate([kt, jnp.zeros((8, LANE), F32)], axis=0)
        if j < N1:
            a1(j)
        else:
            for r0, dup in a2_units[(j - N1) * a2_split:(j - N1 + 1) * a2_split]:
                a2_group(r0, dup)
        valid = jnp.logical_and(row_t >= HOLE, j * KT + row_t - HOLE < S)
        for b in range(NB):
            v_ref[b] = jnp.where(valid, v[:, b * LANE:(b + 1) * LANE], 0.0).astype(BF16)
        ones = jnp.where(jnp.logical_and(valid, lane_t == DH), 1.0, 0.0)
        for u in range(H):
            hv = (u - 1) % H
            off = (hv % HPB) * DH
            vb = v_ref[hv // HPB].astype(F32)
            if off:
                vb = pltpu.roll(vb, LANE - off, 1)
            wt = jnp.where(lane_t < DH, vb, ones)
            top = jnp.where(row24 < DH, kt[u * DH:u * DH + 24, :], wt[:24])
            wt = jnp.concatenate([top, wt[24:]], axis=0)
            w_ref[u, j] = wt.astype(BF16)

    for j in range(NT):
        b2(j)

    for k in CP_FFT2:
        in_copy[k].wait()
    for k1 in range(N1):
        a3_one(k1)

    lane = lax.broadcasted_iota(jnp.int32, (RC, LANE), 1)
    lane_p = lax.broadcasted_iota(jnp.int32, (PC, LANE), 1)

    def srows(slot, k=None):
        if k is None:
            return slice(slot * RC, (slot + 1) * RC)
        return slice(slot * RC + k * PC, slot * RC + (k + 1) * PC)

    def crows(chunk, k=None):
        if k is None:
            return pl.ds(pl.multiple_of(chunk * RC, RC), RC)
        return pl.ds(pl.multiple_of(chunk * RC + k * PC, PC), PC)

    def finalize_max(slot, k=None):
        ln = lane if k is None else lane_p
        mx = mx_ref[srows(slot, k), :]
        mm = jnp.max(jnp.where(ln >= HOLE, mx, -jnp.inf), axis=1, keepdims=True)
        mb = jnp.broadcast_to(mm, mx.shape)
        m_ref[srows(slot, k), :] = mb
        return jnp.max(mb.reshape(-1, 8, LANE), axis=0)

    def finalize_out(pt, slot, k=None):
        ln = lane if k is None else lane_p
        pp = jnp.maximum(pt - 1, 0)
        hp = pp & (H - 1)
        rows = crows(2 * (pp >> 5) + slot, k)
        blk = hp // HPB
        off = (hp % HPB) * DH
        keep = jnp.logical_and(ln >= off, ln < off + DH)
        acc = mx_ref[srows(slot, k), :]
        l = acc[:, DH:DH + 1]
        r0 = pl.reciprocal(l, approx=True)
        r1 = r0 * (2.0 - l * r0)
        o = pltpu.roll(acc * r1, off, 1)
        old = attn_ref[blk, rows, :].astype(F32)
        attn_ref[blk, rows, :] = jnp.where(keep, o, old).astype(BF16)
        return jnp.max(o.reshape(-1, 8, LANE), axis=0)

    def prep_q(pt, slot, k=None):
        hq = pt & (H - 1)
        rows = crows(2 * jnp.minimum(pt >> 5, 1) + slot, k)
        qblk = hq // HPB
        qsh = (LANE - (hq % HPB) * DH) % LANE
        qr = pltpu.roll(q_ref[qblk, rows, :].astype(F32), qsh, 1)
        qc_ref[srows(slot, k), :] = qr
        return jnp.max(qr.reshape(-1, 8, LANE), axis=0)

    def first(t, c):
        for k in range(N2 // 16):
            a4(t * (N2 // 16) + k)
        rows = pl.ds(pl.multiple_of(t * RC, RC), RC)
        lhs = jnp.where(lane < DH, q_ref[0, rows, :].astype(F32), 0.0).astype(BF16)
        mx = None
        for j in range(NT):
            o = jnp.dot(lhs, w_ref[0, j], preferred_element_type=F32)
            s_ref[j, rows, :] = o
            mx = o if mx is None else jnp.maximum(mx, o)
        mx_ref[rows, :] = jnp.where(lane < HOLE, 1.0, mx)
        return c
    lax.fori_loop(0, 2, first, 0, unroll=True)
    finalize_max(0)
    prep_q(1, 0)

    def tiles(u, slot, zs=None):
        q = qc_ref[srows(slot), :]
        acc = None
        for j in range(NT):
            d = s_ref[j, srows(slot), :] - m_ref[srows(slot), :]
            if zs is not None and j in zs:
                d = d + zs[j]
            lhs = jnp.where(lane < HOLE, q, jnp.exp2(d)).astype(BF16)
            o = jnp.dot(lhs, w_ref[u, j], preferred_element_type=F32)
            s_ref[j, srows(slot), :] = o
            acc = o if acc is None else jnp.where(lane < HOLE, acc + o, jnp.maximum(acc, o))
        mx_ref[srows(slot), :] = acc

    def filler(pt_out, pt_q, slot, fenced):
        zs = {}
        for k in range(NPC):
            tok = (finalize_max(slot, k) + finalize_out(pt_out, slot, k)
                   + prep_q(pt_q, slot, k))
            if fenced and FENCE0 + FENCED * k < NT:
                zs[FENCE0 + FENCED * k] = jnp.minimum(
                    jnp.abs(jnp.max(tok, axis=0, keepdims=True)), 0.0)
        return zs

    def main(i, c):
        for half in range(2):
            pt = 2 * i + 1 + half
            u = pt & (H - 1)
            tiles(u, 0, filler(pt - 1, pt, 1, True))
            tiles(u, 1, filler(pt, pt + 1, 0, half == 0))
        return c
    nsteps = H
    lax.fori_loop(0, nsteps, main, 0)
    finalize_out(2 * H, 1)

    def out_copy(i):
        rows = pl.ds(pl.multiple_of(i * RO, RO), RO)
        return pltpu.make_async_copy(out_ref.at[rows], out_hbm.at[rows], sem_out.at[i])

    def b3(i, c):
        for sub in range(RO // R5):
            rows = pl.ds(pl.multiple_of(i * RO + sub * R5, R5), R5)

            def proj():
                a = jnp.concatenate([attn_ref[b, rows, :] for b in range(NB)], axis=1)
                y = jnp.dot(a, wop_ref[...], preferred_element_type=F32)
                out_ref[rows, DP:] = y[:, LANE:].astype(BF16)
                return y[:, :LANE]
            a5(rows, proj)
        out_copy(i).start()
        return c
    lax.fori_loop(0, S // RO, b3, 0, unroll=2)

    for i in range(S // RO):
        out_copy(i).wait()


@jax.jit
def pallas_concat_heads__spectral_gfnet__mha_block__prompt_kernel(
    A_x: jax.Array,
    A_w_r: jax.Array,
    A_w_i: jax.Array,
    B_x: jax.Array,
    B_wqkv: jax.Array,
    B_wo: jax.Array,
):
    m1, m2, g, gi = _fft_constants()
    vm = pltpu.VMEM
    scratch = [
        vm((D, S), BF16),
        vm((DF, S), BF16),
        vm((DF, S), BF16),
        vm((D, S), BF16),
        vm((D, 3 * D), BF16),
        vm((DP, D), BF16),
        vm((NG, 2 * M, 2 * M), BF16),
        vm((NG, 2 * M, 2 * M), BF16),
        vm((N1, 2 * N2, 2 * N2), BF16),
        vm((N1, 2 * N2, 2 * N2), BF16),
        vm((S, 2 * D), BF16),
        pltpu.SemaphoreType.DMA((NBK,)),
        pltpu.SemaphoreType.DMA((10,)),
        pltpu.SemaphoreType.DMA((S // RO,)),
        vm((2 * FR, S), F32),
        vm((NG, 2 * M, LANE), BF16),
        vm((2, 320, LANE), F32),
        vm((N1, FP, 2 * N2), F32),
        vm((N1, 2 * N2, FP), F32),
        vm((S, DP), F32),
        vm((2, FP // LANE, S, LANE), F32),
        vm((S, D), BF16),
        vm((SP, D), BF16),
        vm((DP, DP), BF16),
        vm((DP, DP), BF16),
        vm((DP, D), BF16),
        vm((DP, DP), BF16),
        vm((NB, S, LANE), BF16),
        vm((NB, LANE, LANE), BF16),
        vm((H, NT, LANE, LANE), BF16),
        vm((NT, 2 * RC, LANE), F32),
        vm((2 * RC, LANE), F32),
        vm((2 * RC, LANE), F32),
        vm((2 * RC, LANE), F32),
        vm((NB, S, LANE), BF16),
    ]
    any_spec = pl.BlockSpec(memory_space=pl.ANY)
    out = pl.pallas_call(
        _kernel,
        out_shape=jax.ShapeDtypeStruct((S, 2 * D), BF16),
        in_specs=[any_spec] * 10,
        out_specs=any_spec,
        scratch_shapes=scratch,
        compiler_params=pltpu.CompilerParams(vmem_limit_bytes=120 * 2**20),
    )(A_x.reshape(S, D).T, A_w_r.T, A_w_i.T, B_x.reshape(S, D).T, B_wqkv, B_wo,
      m1, m2, g, gi)
    return out.reshape(1, S, 2 * D)
```
